```python
import jax
import jax.numpy as jnp

def _softmax(x, axis=-1):
    return jax.nn.softmax(x, axis=axis)
def _gelu(x):
    return jax.nn.gelu(x, approximate=True)
def _silu(x):
    return jax.nn.silu(x)
def _sigmoid(x):
    return jax.nn.sigmoid(x)
def _layernorm(x, axis=-1, eps=1e-5):
    m = jnp.mean(x, axis=axis, keepdims=True)
    v = jnp.var(x, axis=axis, keepdims=True)
    return (x - m) / jnp.sqrt(v + eps)
def _scatter_add(tgt, idx, src, axis=0):
    return tgt.at[idx].add(src)
def _segment_sum(src, seg, n):
    return jax.ops.segment_sum(src, seg, n)
class _Rng:
    def __init__(self, key):
        self._k = key
    def _next(self):
        self._k, sub = jax.random.split(self._k)
        return sub
    def normal(self, shape):
        return jax.random.normal(self._next(), shape, dtype=jnp.bfloat16)
    def randint(self, lo, hi, shape):
        return jax.random.randint(self._next(), shape, lo, hi, dtype=jnp.int32)
    def uniform(self, shape, lo=0.0, hi=1.0):
        return jax.random.uniform(self._next(), shape, jnp.bfloat16, lo, hi)
    def permutation(self, n):
        return jax.random.permutation(self._next(), n)


kernel_name = 'gated_mix__mha_block_cached__moe_arch_mod__decode'

def setup_inputs():
    _rng = _Rng(jax.random.key(int.from_bytes(__import__("os").urandom(4), "little")))
    _w = (lambda a: (lambda t: t.astype(jnp.bfloat16) if jnp.issubdtype(t.dtype, jnp.floating) else t)(jnp.asarray(a)))
    def _A_setup():
        B, Sq, D = 4, 1, 1024
        H, Sk, Dh = 32, 8192, 128
        return {
            "x": _w((lambda *s: _rng.normal(s) * 0.05)(B, Sq, D)),
            "k_cache": _w((lambda *s: _rng.normal(s) * 0.05)(B, H, Sk, Dh)),
            "v_cache": _w((lambda *s: _rng.normal(s) * 0.05)(B, H, Sk, Dh)),
            "wq": _w((lambda *s: _rng.normal(s) * 0.05)(D, H * Dh) * (D ** -0.5)),
            "wo": _w((lambda *s: _rng.normal(s) * 0.05)(H * Dh, D) * ((H * Dh) ** -0.5)),
        }
    _A_in = _A_setup()

    def _B_setup():
        B, S, D, F, C = 4, 1, 1024, 3584, 1
        return {
            "x": _w((lambda *s: _rng.normal(s) * 0.05)(B, S, D)),
            "w_r": _w((lambda *s: _rng.normal(s) * 0.05)(D)),
            "w_gate": _w((lambda *s: _rng.normal(s) * 0.05)(D, F)),
            "w_up": _w((lambda *s: _rng.normal(s) * 0.05)(D, F)),
            "w_down": _w((lambda *s: _rng.normal(s) * 0.05)(F, D)),
        }
    _B_in = _B_setup()

    return {
        "A_x": _A_in["x"],
        "A_k_cache": _A_in["k_cache"],
        "A_v_cache": _A_in["v_cache"],
        "A_wq": _A_in["wq"],
        "A_wo": _A_in["wo"],
        "B_x": _B_in["x"],
        "B_w_r": _B_in["w_r"],
        "B_w_gate": _B_in["w_gate"],
        "B_w_up": _B_in["w_up"],
        "B_w_down": _B_in["w_down"],
        "gate_w": _w((lambda *s: _rng.normal(s) * 0.05)(1024)),
    }

def reference(A_x, A_k_cache, A_v_cache, A_wq, A_wo, B_x, B_w_r, B_w_gate, B_w_up, B_w_down, gate_w):
    def _A_ref(x, k_cache, v_cache, wq, wo):
        B, Sq, D = x.shape
        H, Dh = 32, 128
        q = (lambda x, *d: x.transpose(*d))((x @ wq).reshape(B, Sq, H, Dh), 0, 2, 1, 3)
        scores = jnp.einsum("bhqd,bhkd->bhqk", q, k_cache) * (Dh ** -0.5)
        p = _softmax(scores, axis=-1)
        o = jnp.einsum("bhqk,bhkd->bhqd", p, v_cache)
        return (lambda x, *d: x.transpose(*d))(o, 0, 2, 1, 3).reshape(B, Sq, H * Dh) @ wo

    def _B_ref(x, w_r, w_gate, w_up, w_down):
        B, S, D = x.shape
        C = 1
        r = x @ w_r
        idx = jnp.argsort(-r, axis=-1)[:, :C]
        idx_e = jnp.repeat(idx.reshape(B, C, 1), D, axis=2)
        x_sel = jnp.take_along_axis(x, idx_e, axis=1)
        g = _silu(x_sel @ w_gate)
        u = x_sel @ w_up
        y = (g * u) @ w_down
        r_sel = _sigmoid(jnp.take_along_axis(r, idx, axis=1))
        y = y * r_sel.reshape(B, C, 1)
        b_off = (jnp.arange(B) * S).reshape(B, 1)
        flat_idx = (idx + b_off).reshape(B * C)
        zero = (x * 0.0).reshape(B * S, D)
        upd = _scatter_add(zero, flat_idx, y.reshape(B * C, D), axis=0)
        return x + upd.reshape(B, S, D)

    x = A_x
    g = _sigmoid((x * gate_w).sum(-1, keepdims=True))
    a = _A_ref(x, A_k_cache, A_v_cache, A_wq, A_wo)
    b = _B_ref(x, B_w_r, B_w_gate, B_w_up, B_w_down)
    return g * a + (1 - g) * b
```

```python
import jax
import jax.numpy as jnp
from jax import lax
import jax.experimental.pallas as pl
import jax.experimental.pallas.tpu as pltpu


def _sigmoid(z):
    return 1.0 / (1.0 + jnp.exp(-z))


@jax.jit
def pallas_gated_mix__mha_block_cached__moe_arch_mod__decode_kernel(
    A_x, A_k_cache, A_v_cache, A_wq, A_wo, B_x, B_w_r, B_w_gate, B_w_up, B_w_down, gate_w,
):
    B, Sq, D = A_x.shape
    _, H, Sk, Dh = A_k_cache.shape
    F = B_w_gate.shape[1]
    FC = 128
    NF = F // FC
    scale = Dh ** -0.5
    f32, bf16 = jnp.float32, jnp.bfloat16

    def kernel(ax_ref, wr_ref, gw_ref, k_ref, v_ref, wq_ref, wo_ref, wg_ref, wu_ref, wd_ref,
               out_ref, q_scr, o_scr, a_acc, y_acc):
        h = pl.program_id(0)
        b = pl.program_id(1)
        step = h * B + b

        @pl.when(step == 0)
        def _():
            a_acc[...] = jnp.zeros_like(a_acc)
            y_acc[...] = jnp.zeros_like(y_acc)

        @pl.when(b == 0)
        def _():
            q_scr[...] = jnp.dot(ax_ref[...], wq_ref[...], preferred_element_type=f32)
            o_scr[...] = jnp.zeros_like(o_scr)

        q = q_scr[...].astype(bf16)
        s = lax.dot_general(q, k_ref[...], (((1,), (1,)), ((), ())), preferred_element_type=f32) * scale
        m = jnp.max(s, axis=-1, keepdims=True)
        p = jnp.exp(s - m)
        l = jnp.sum(p, axis=-1, keepdims=True)
        o = jnp.dot(p.astype(bf16), v_ref[...], preferred_element_type=f32) / l
        row = lax.broadcasted_iota(jnp.int32, o.shape, 0)
        o_scr[...] = jnp.where(row == b, o, o_scr[...])

        @pl.when(b == B - 1)
        def _():
            a_acc[...] += jnp.dot(o_scr[...].astype(bf16), wo_ref[...], preferred_element_type=f32)

        @pl.when(step < NF)
        def _():
            xb = ax_ref[...]
            g = jnp.dot(xb, wg_ref[...], preferred_element_type=f32)
            u = jnp.dot(xb, wu_ref[...], preferred_element_type=f32)
            hh = (g * _sigmoid(g)) * u
            y_acc[...] += jnp.dot(hh.astype(bf16), wd_ref[...], preferred_element_type=f32)

        @pl.when(step == H * B - 1)
        def _():
            xa = ax_ref[...].astype(f32)
            xb = xa
            gate = _sigmoid(jnp.sum(xa * gw_ref[...].astype(f32), axis=-1, keepdims=True))
            r = jnp.sum(xb * wr_ref[...].astype(f32), axis=-1, keepdims=True)
            y = y_acc[...] * _sigmoid(r)
            bb = xb + (xb * 0.0 + y)
            out_ref[...] = (gate * a_acc[...] + (1.0 - gate) * bb).astype(out_ref.dtype)

    full = lambda shape: pl.BlockSpec(shape, lambda h, b: (0,) * len(shape))
    fidx = lambda h, b: jnp.minimum(h * B + b, NF - 1)
    out = pl.pallas_call(
        kernel,
        grid=(H, B),
        in_specs=[
            full((B, D)), full((1, D)), full((1, D)),
            pl.BlockSpec((None, None, Sk, Dh), lambda h, b: (b, h, 0, 0)),
            pl.BlockSpec((None, None, Sk, Dh), lambda h, b: (b, h, 0, 0)),
            pl.BlockSpec((D, Dh), lambda h, b: (0, h)),
            pl.BlockSpec((Dh, D), lambda h, b: (h, 0)),
            pl.BlockSpec((D, FC), lambda h, b: (0, fidx(h, b))),
            pl.BlockSpec((D, FC), lambda h, b: (0, fidx(h, b))),
            pl.BlockSpec((FC, D), lambda h, b: (fidx(h, b), 0)),
        ],
        out_specs=full((B, D)),
        out_shape=jax.ShapeDtypeStruct((B, D), A_x.dtype),
        scratch_shapes=[
            pltpu.VMEM((B, Dh), f32), pltpu.VMEM((B, Dh), f32),
            pltpu.VMEM((B, D), f32), pltpu.VMEM((B, D), f32),
        ],
        compiler_params=pltpu.CompilerParams(
            dimension_semantics=("arbitrary", "arbitrary"),
            vmem_limit_bytes=64 * 1024 * 1024,
        ),
    )(A_x.reshape(B, D), B_w_r.reshape(1, D), gate_w.reshape(1, D),
      A_k_cache, A_v_cache, A_wq, A_wo, B_w_gate, B_w_up, B_w_down)
    return out.reshape(B, Sq, D)
```

```python
import jax
import jax.numpy as jnp
from jax import lax
import jax.experimental.pallas as pl
import jax.experimental.pallas.tpu as pltpu


def _sigmoid(z):
    return 1.0 / (1.0 + jnp.exp(-z))


NS = 4
CR = 128
G = 1
VS = 1
small1d = True


@jax.jit
def pallas_gated_mix__mha_block_cached__moe_arch_mod__decode_kernel(A_x, A_k_cache, A_v_cache, A_wq, A_wo, B_x, B_w_r, B_w_gate, B_w_up, B_w_down, gate_w):
  B, Sq, D = A_x.shape
  _, H, Sk, Dh = A_k_cache.shape
  F = B_w_gate.shape[1]
  NSTEP = B * H
  FC = 512
  NF = F // FC
  FSTEPS = 16
  FR = D // FSTEPS
  DR = FC // FSTEPS
  WOR = Dh // B
  NC = Sk // CR
  GR = Sk // G
  CPG = NC // (2 * G)
  scale = Dh ** -0.5
  f32, bf16 = jnp.float32, jnp.bfloat16

  def kernel(x_ref, wr_ref, gw_ref, k_hbm, v_hbm, wq_hbm, wo_hbm, wg_hbm, wu_hbm, wd_hbm,
             out_ref, kbuf, vbuf, wq_buf, wo_buf, wg_buf, wu_buf, wd_buf,
             q_scr, s_scr, o_scr, a_acc, y_acc, ksem, vsem, xsem, fsem, qsem):

    def kv_chunk(step, slot, c):
      h = step // B
      b = step % B
      rows = pl.ds(c * CR, CR)
      pltpu.make_async_copy(k_hbm.at[b, h, rows], kbuf.at[slot, rows], ksem.at[slot]).start(priority=0)
      pltpu.make_async_copy(v_hbm.at[b, h, rows], vbuf.at[slot, rows], vsem.at[slot]).start(priority=1)

    def wo_copies(step):
      r0 = pl.multiple_of(step * WOR, WOR)
      return [pltpu.make_async_copy(wo_hbm.at[pl.ds(r0 + i * 16, 16)], wo_buf.at[pl.ds(r0 + i * 16, 16)],
                                    xsem.at[step % NS]) for i in range(WOR // 16)]

    def ffn_copies(step):
      j = step // FSTEPS
      r = step % FSTEPS
      c0 = pl.multiple_of(j * FC, FC)
      cps = []
      for i in range(2):
        rr = pl.ds(pl.multiple_of(r * FR + i * (FR // 2), FR // 2), FR // 2)
        cps.append(pltpu.make_async_copy(wg_hbm.at[rr, pl.ds(c0, FC)], wg_buf.at[j, rr], fsem.at[step % NS]))
        cps.append(pltpu.make_async_copy(wu_hbm.at[rr, pl.ds(c0, FC)], wu_buf.at[j, rr], fsem.at[step % NS]))
      for i in range(2):
        rr = pl.ds(pl.multiple_of(step * DR + i * (DR // 2), DR // 2), DR // 2)
        cps.append(pltpu.make_async_copy(wd_hbm.at[rr], wd_buf.at[rr], fsem.at[step % NS]))
      return cps

    def start_extras(step):
      for i, cp in enumerate(wo_copies(step)):
        cp.start(priority=i % 2)

      @pl.when(step < NF * FSTEPS)
      def _():
        for i, cp in enumerate(ffn_copies(step)):
          cp.start(priority=i % 2)

    def wq_start(i, c):
      r = pl.ds(pl.multiple_of(i * 16, 16), 16)
      for t in range(4):
        cs = pl.ds(t * 1024, 1024)
        pltpu.make_async_copy(wq_hbm.at[r, cs], wq_buf.at[r, cs], qsem.at[0]).start(priority=t % 2)
      return c
    lax.fori_loop(0, D // 16, wq_start, 0)

    def pro(step, c):
      def pc(cc, c2):
        kv_chunk(step, step, cc)
        return c2
      lax.fori_loop(0, NC, pc, 0)
      start_extras(step)
      return c
    lax.fori_loop(0, NS - 1, pro, 0)

    a_acc[...] = jnp.zeros_like(a_acc)
    y_acc[...] = jnp.zeros_like(y_acc)
    o_scr[...] = jnp.zeros_like(o_scr)
    pltpu.make_async_copy(wq_hbm, wq_buf, qsem.at[0]).wait()
    x = x_ref[...]
    for hh in range(H):
      q_scr[hh] = jnp.dot(x, wq_buf[:, hh * Dh:(hh + 1) * Dh], preferred_element_type=f32)

    def body(step, carry):
      h = step // B
      b = step % B
      slot = step % NS
      nxt = step + NS - 1
      nslot = nxt % NS
      more = nxt < NSTEP

      def issue(g):
        @pl.when(more)
        def _():
          for c in range(g * CPG, (g + 1) * CPG):
            kv_chunk(nxt, nslot, c)

      q = q_scr[h].astype(bf16)
      pltpu.make_async_copy(k_hbm.at[0, 0], kbuf.at[slot], ksem.at[slot]).wait()
      for g in range(G):
        issue(g)
        s_scr[:, g * GR:(g + 1) * GR] = lax.dot_general(
            q, kbuf[slot, g * GR:(g + 1) * GR, :], (((1,), (1,)), ((), ())),
            preferred_element_type=f32) * scale
      s = s_scr[...]
      m = jnp.max(s, axis=-1, keepdims=True)
      p = jnp.exp(s - m)
      l = jnp.sum(p, axis=-1, keepdims=True)
      pb = p.astype(bf16)
      pltpu.make_async_copy(v_hbm.at[0, 0], vbuf.at[slot], vsem.at[slot]).wait()
      o = jnp.zeros((B, Dh), f32)
      for g in range(G):
        issue(G + g)
        o = o + jnp.dot(pb[:, g * GR:(g + 1) * GR], vbuf[slot, g * GR:(g + 1) * GR, :],
                        preferred_element_type=f32)
      o = o / l
      row = lax.broadcasted_iota(jnp.int32, o.shape, 0)
      o_scr[...] = jnp.where(row == b, o, o_scr[...])

      @pl.when(more)
      def _():
        start_extras(nxt)

      for cp in wo_copies(step):
        cp.wait()

      @pl.when(step < NF * FSTEPS)
      def _():
        for cp in ffn_copies(step):
          cp.wait()

      @pl.when(b == B - 1)
      def _():
        w = wo_buf[pl.ds(pl.multiple_of(h * Dh, Dh), Dh), :]
        a_acc[...] += jnp.dot(o_scr[...].astype(bf16), w, preferred_element_type=f32)

      @pl.when(jnp.logical_and(step % FSTEPS == FSTEPS - 1, step < NF * FSTEPS))
      def _():
        j = step // FSTEPS
        xb = x_ref[...]
        gg = jnp.dot(xb, wg_buf[j], preferred_element_type=f32)
        uu = jnp.dot(xb, wu_buf[j], preferred_element_type=f32)
        hid = (gg * _sigmoid(gg)) * uu
        wdj = wd_buf[pl.ds(pl.multiple_of(j * FC, FC), FC), :]
        y_acc[...] += jnp.dot(hid.astype(bf16), wdj, preferred_element_type=f32)
      return carry

    lax.fori_loop(0, NSTEP, body, 0)

    xa = x_ref[...].astype(f32)
    gw = gw_ref[...].astype(f32).reshape(1, D)
    wr = wr_ref[...].astype(f32).reshape(1, D)
    gate = _sigmoid(jnp.sum(xa * gw, axis=-1, keepdims=True))
    r = jnp.sum(xa * wr, axis=-1, keepdims=True)
    y = y_acc[...] * _sigmoid(r)
    bb = xa + (xa * 0.0 + y)
    out_ref[...] = (gate * a_acc[...] + (1.0 - gate) * bb).astype(out_ref.dtype)

  vm = pl.BlockSpec(memory_space=pltpu.VMEM)
  hbm = pl.BlockSpec(memory_space=pl.ANY)
  wr_in, gw_in = (B_w_r, gate_w) if small1d else (B_w_r.reshape(1, D), gate_w.reshape(1, D))
  out = pl.pallas_call(
      kernel,
      in_specs=[vm, vm, vm] + [hbm] * 7,
      out_specs=vm,
      out_shape=jax.ShapeDtypeStruct((B, D), A_x.dtype),
      scratch_shapes=[
          pltpu.VMEM((NS, Sk, Dh), bf16), pltpu.VMEM((NS, Sk, Dh), bf16),
          pltpu.VMEM((D, H * Dh), bf16), pltpu.VMEM((H * Dh, D), bf16),
          pltpu.VMEM((NF, D, FC), bf16), pltpu.VMEM((NF, D, FC), bf16), pltpu.VMEM((F, D), bf16),
          pltpu.VMEM((H, B, Dh), f32), pltpu.VMEM((B, Sk), f32), pltpu.VMEM((B, Dh), f32),
          pltpu.VMEM((B, D), f32), pltpu.VMEM((B, D), f32),
          pltpu.SemaphoreType.DMA((NS,)), pltpu.SemaphoreType.DMA((NS,)),
          pltpu.SemaphoreType.DMA((NS,)), pltpu.SemaphoreType.DMA((NS,)), pltpu.SemaphoreType.DMA((1,)),
      ],
      compiler_params=pltpu.CompilerParams(vmem_limit_bytes=110 * 1024 * 1024),
  )(A_x.reshape(B, D), wr_in, gw_in, A_k_cache, A_v_cache, A_wq, A_wo, B_w_gate, B_w_up, B_w_down)
  return out.reshape(B, Sq, D)
```

```python
import jax
import jax.numpy as jnp
from jax import lax
import jax.experimental.pallas as pl
import jax.experimental.pallas.tpu as pltpu


def _sigmoid(z):
    return 1.0 / (1.0 + jnp.exp(-z))


NS = 3
CH = (192, 64, 192, 64, 192, 64, 192, 64, 192, 64, 192, 64, 192, 64, 192, 64)
R = 4
PAT = 'hn'
mode = 'full'


@jax.jit
def pallas_gated_mix__mha_block_cached__moe_arch_mod__decode_kernel(A_x, A_k_cache, A_v_cache, A_wq, A_wo, B_x, B_w_r, B_w_gate, B_w_up, B_w_down, gate_w):
  B, Sq, D = A_x.shape
  _, H, Sk, Dh = A_k_cache.shape
  F = B_w_gate.shape[1]
  NSTEP = B * H
  FC = 512
  NF = F // FC
  FSTEPS = 16
  FR = D // FSTEPS
  DR = FC // FSTEPS
  WOR = Dh // B
  RR = Sk // R
  SCHED = []
  if PAT == 'hn':
    assert sum(CH) == RR
    for i, n in enumerate(CH):
      for g in range(R):
        o = g * RR + sum(CH[:i])
        SCHED += [(0, o, n, 0), (1, o, n, 1)]
  else:
    assert 2 * sum(CH) == RR
    for i, n in enumerate(CH):
      for g in range(R):
        o = g * RR + 2 * sum(CH[:i])
        SCHED += [(0, o, n, 0), (0, o + n, n, 1), (1, o, n, 0), (1, o + n, n, 1)]
  NC = len(SCHED)
  G = 1
  GR = Sk
  scale = Dh ** -0.5
  f32, bf16 = jnp.float32, jnp.bfloat16

  def kernel(x_ref, wr_ref, gw_ref, k_hbm, v_hbm, wq_hbm, wo_hbm, wg_hbm, wu_hbm, wd_hbm,
             out_ref, kbuf, vbuf, wq_buf, wo_buf, wg_buf, wu_buf, wd_buf,
             q_scr, s_scr, o_scr, a_acc, y_acc, ksem, vsem, xsem, fsem, qsem):

    def kv_chunk(step, slot, c):
      h = step // B
      b = step % B
      t, o, n, pr = SCHED[c]
      rows = pl.ds(o, n)
      src, dst, sem = ((k_hbm, kbuf, ksem), (v_hbm, vbuf, vsem))[t]
      pltpu.make_async_copy(src.at[b, h, rows], dst.at[slot, rows], sem.at[slot]).start(priority=pr)

    def wo_copies(step):
      r0 = pl.multiple_of(step * WOR, WOR)
      return [pltpu.make_async_copy(wo_hbm.at[pl.ds(r0 + i * 16, 16)], wo_buf.at[pl.ds(r0 + i * 16, 16)],
                                    xsem.at[step % NS]) for i in range(WOR // 16)]

    def ffn_copies(step):
      j = step // FSTEPS
      r = step % FSTEPS
      c0 = pl.multiple_of(j * FC, FC)
      cps = []
      for i in range(2):
        rr = pl.ds(pl.multiple_of(r * FR + i * (FR // 2), FR // 2), FR // 2)
        cps.append(pltpu.make_async_copy(wg_hbm.at[rr, pl.ds(c0, FC)], wg_buf.at[j, rr], fsem.at[step % NS]))
        cps.append(pltpu.make_async_copy(wu_hbm.at[rr, pl.ds(c0, FC)], wu_buf.at[j, rr], fsem.at[step % NS]))
      for i in range(2):
        rr = pl.ds(pl.multiple_of(step * DR + i * (DR // 2), DR // 2), DR // 2)
        cps.append(pltpu.make_async_copy(wd_hbm.at[rr], wd_buf.at[rr], fsem.at[step % NS]))
      return cps

    def start_extras(step):
      for i, cp in enumerate(wo_copies(step)):
        cp.start(priority=i % 2)

      @pl.when(step < NF * FSTEPS)
      def _():
        for i, cp in enumerate(ffn_copies(step)):
          cp.start(priority=i % 2)

    def wq_start(i, c):
      r = pl.ds(pl.multiple_of(i * 16, 16), 16)
      for t in range(4):
        cs = pl.ds(t * 1024, 1024)
        pltpu.make_async_copy(wq_hbm.at[r, cs], wq_buf.at[r, cs], qsem.at[0]).start(priority=t % 2)
      return c
    lax.fori_loop(0, D // 16, wq_start, 0)

    def pro(step, c):
      for cc in range(NC):
        kv_chunk(step, step, cc)
      start_extras(step)
      return c
    lax.fori_loop(0, NS - 1, pro, 0)

    a_acc[...] = jnp.zeros_like(a_acc)
    y_acc[...] = jnp.zeros_like(y_acc)
    o_scr[...] = jnp.zeros_like(o_scr)
    pltpu.make_async_copy(wq_hbm, wq_buf, qsem.at[0]).wait()
    x = x_ref[...]
    for hh in range(H):
      q_scr[hh] = jnp.dot(x, wq_buf[:, hh * Dh:(hh + 1) * Dh], preferred_element_type=f32)

    def body(step, carry):
      h = step // B
      b = step % B
      slot = step % NS
      nxt = step + NS - 1
      nslot = nxt % NS
      more = nxt < NSTEP

      def issue(g):
        @pl.when(more)
        def _():
          for c in range(g * NC // 2, (g + 1) * NC // 2):
            kv_chunk(nxt, nslot, c)

      q = q_scr[h].astype(bf16)
      pltpu.make_async_copy(k_hbm.at[0, 0], kbuf.at[slot], ksem.at[slot]).wait()
      for g in range(G):
        issue(g)
        if mode == 'full': s_scr[:, g * GR:(g + 1) * GR] = lax.dot_general(
            q, kbuf[slot, g * GR:(g + 1) * GR, :], (((1,), (1,)), ((), ())),
            preferred_element_type=f32) * scale
      s = s_scr[...]
      m = jnp.max(s, axis=-1, keepdims=True)
      p = jnp.exp(s - m)
      l = jnp.sum(p, axis=-1, keepdims=True)
      pb = p.astype(bf16)
      pltpu.make_async_copy(v_hbm.at[0, 0], vbuf.at[slot], vsem.at[slot]).wait()
      o = jnp.zeros((B, Dh), f32)
      for g in range(G):
        issue(G + g)
        if mode == 'full': o = o + jnp.dot(pb[:, g * GR:(g + 1) * GR], vbuf[slot, g * GR:(g + 1) * GR, :],
                        preferred_element_type=f32)
      o = o / l
      row = lax.broadcasted_iota(jnp.int32, o.shape, 0)
      o_scr[...] = jnp.where(row == b, o, o_scr[...])

      @pl.when(more)
      def _():
        start_extras(nxt)

      for cp in wo_copies(step):
        cp.wait()

      @pl.when(step < NF * FSTEPS)
      def _():
        for cp in ffn_copies(step):
          cp.wait()

      @pl.when(b == B - 1 if mode == 'full' else b == 77)
      def _():
        w = wo_buf[pl.ds(pl.multiple_of(h * Dh, Dh), Dh), :]
        a_acc[...] += jnp.dot(o_scr[...].astype(bf16), w, preferred_element_type=f32)

      @pl.when(jnp.logical_and(step % FSTEPS == (FSTEPS - 1 if mode == 'full' else 77), step < NF * FSTEPS))
      def _():
        j = step // FSTEPS
        xb = x_ref[...]
        gg = jnp.dot(xb, wg_buf[j], preferred_element_type=f32)
        uu = jnp.dot(xb, wu_buf[j], preferred_element_type=f32)
        hid = (gg * _sigmoid(gg)) * uu
        wdj = wd_buf[pl.ds(pl.multiple_of(j * FC, FC), FC), :]
        y_acc[...] += jnp.dot(hid.astype(bf16), wdj, preferred_element_type=f32)
      return carry

    lax.fori_loop(0, NSTEP, body, 0)

    xa = x_ref[...].astype(f32)
    gw = gw_ref[...].astype(f32).reshape(1, D)
    wr = wr_ref[...].astype(f32).reshape(1, D)
    gate = _sigmoid(jnp.sum(xa * gw, axis=-1, keepdims=True))
    r = jnp.sum(xa * wr, axis=-1, keepdims=True)
    y = y_acc[...] * _sigmoid(r)
    bb = xa + (xa * 0.0 + y)
    out_ref[...] = (gate * a_acc[...] + (1.0 - gate) * bb).astype(out_ref.dtype)

  vm = pl.BlockSpec(memory_space=pltpu.VMEM)
  hbm = pl.BlockSpec(memory_space=pl.ANY)
  wr_in, gw_in = B_w_r, gate_w
  out = pl.pallas_call(
      kernel,
      in_specs=[vm, vm, vm] + [hbm] * 7,
      out_specs=vm,
      out_shape=jax.ShapeDtypeStruct((B, D), A_x.dtype),
      scratch_shapes=[
          pltpu.VMEM((NS, Sk, Dh), bf16), pltpu.VMEM((NS, Sk, Dh), bf16),
          pltpu.VMEM((D, H * Dh), bf16), pltpu.VMEM((H * Dh, D), bf16),
          pltpu.VMEM((NF, D, FC), bf16), pltpu.VMEM((NF, D, FC), bf16), pltpu.VMEM((F, D), bf16),
          pltpu.VMEM((H, B, Dh), f32), pltpu.VMEM((B, Sk), f32), pltpu.VMEM((B, Dh), f32),
          pltpu.VMEM((B, D), f32), pltpu.VMEM((B, D), f32),
          pltpu.SemaphoreType.DMA((NS,)), pltpu.SemaphoreType.DMA((NS,)),
          pltpu.SemaphoreType.DMA((NS,)), pltpu.SemaphoreType.DMA((NS,)), pltpu.SemaphoreType.DMA((1,)),
      ],
      compiler_params=pltpu.CompilerParams(vmem_limit_bytes=110 * 1024 * 1024),
  )(A_x.reshape(B, D), wr_in, gw_in, A_k_cache, A_v_cache, A_wq, A_wo, B_w_gate, B_w_up, B_w_down)
  return out.reshape(B, Sq, D)
```

```python
import jax
import jax.numpy as jnp
from jax import lax
import jax.experimental.pallas as pl
import jax.experimental.pallas.tpu as pltpu


def _sigmoid(z):
    return 1.0 / (1.0 + jnp.exp(-z))


NS = 3
CH = (192, 64)
R = 4
GC = 2560
U0 = 2
US = 4
mode = 'full'


@jax.jit
def pallas_gated_mix__mha_block_cached__moe_arch_mod__decode_kernel(A_x, A_k_cache, A_v_cache, A_wq, A_wo, B_x, B_w_r, B_w_gate, B_w_up, B_w_down, gate_w):
  B, Sq, D = A_x.shape
  _, H, Sk, Dh = A_k_cache.shape
  F = B_w_gate.shape[1]
  NSTEP = B * H
  FC = 512
  NF = F // FC
  RR = Sk // R
  PER = sum(CH)
  scale = Dh ** -0.5
  f32, bf16 = jnp.float32, jnp.bfloat16
  NU = 8
  F0 = U0 + NU * US + NS

  def kernel(x_ref, wr_ref, gw_ref, k_hbm, v_hbm, wq_hbm, wo_hbm, wg_hbm, wu_hbm, wd_hbm,
             out_ref, kbuf, vbuf, wq_buf, wo_buf, wg_buf, wu_buf, wd_buf,
             q_scr, o_scr, a_acc, y_acc, ksem, vsem, wsem):

    def kv_issue(step, slot, lo, hi):
      h = step % H
      b = step // H
      for i in range(lo, hi):
        o0 = 0
        for n in CH:
          for g in range(R):
            rows = pl.ds(g * RR + i * PER + o0, n)
            pltpu.make_async_copy(k_hbm.at[b, h, rows], kbuf.at[slot, rows], ksem.at[slot]).start(priority=0)
            pltpu.make_async_copy(v_hbm.at[b, h, rows], vbuf.at[slot, rows], vsem.at[slot]).start(priority=1)
          o0 += n

    NI = RR // PER

    def weight_unit(pair, starts, region, slab, pieces, sem_i):
      def it(i, c):
        for (dr, nr, c0, nc) in pieces:
          for g in range(R):
            for t in range(2):
              src, dst = pair[t]
              rows = pl.ds(pl.multiple_of(starts[t] + g * region + i * slab + dr, 8), nr)
              cols = pl.ds(c0, nc)
              pltpu.make_async_copy(src.at[rows, cols], dst.at[rows, cols], wsem.at[sem_i]).start(priority=t)
        return c
      lax.fori_loop(0, region // slab, it, 0)

    wqp = ((wq_hbm, wq_buf),) * 2
    wop = ((wo_hbm, wo_buf),) * 2
    wdp = ((wd_hbm, wd_buf),) * 2
    wgp = ((wg_hbm, wg_buf), (wu_hbm, wu_buf))
    rowp = ((0, 24, 0, D), (24, 8, 0, D))
    for u in range(2):
      weight_unit(wqp, (u * 512, u * 512 + 256), 64, 8, ((0, 8, 0, 3072), (0, 8, 3072, 1024)), 0)

    def late_unit(u):
      if u < 2:
        weight_unit(wop, (u * 2048, u * 2048 + 1024), 256, 32, rowp, 1)
      elif u < 6:
        weight_unit(wgp, ((u - 2) * 256,) * 2, 64, 8, ((0, 8, 0, GC), (0, 8, GC, F - GC)), 1)
      else:
        weight_unit(wdp, ((u - 6) * 1792, (u - 6) * 1792 + 896), 224, 32, rowp, 1)

    def pro(step, c):
      kv_issue(step, step, 0, NI)
      return c
    lax.fori_loop(0, NS - 1, pro, 0)

    a_acc[...] = jnp.zeros_like(a_acc)
    y_acc[...] = jnp.zeros_like(y_acc)
    o_scr[...] = jnp.zeros_like(o_scr)
    pltpu.make_async_copy(wq_hbm, wq_buf, wsem.at[0]).wait()
    x = x_ref[...]
    for hh in range(H):
      q_scr[hh] = jnp.dot(x, wq_buf[:, hh * Dh:(hh + 1) * Dh], preferred_element_type=f32)

    def body(step, carry):
      h = step % H
      b = step // H
      slot = step % NS
      nxt = step + NS - 1
      nslot = nxt % NS
      more = nxt < NSTEP

      q = q_scr[h].astype(bf16)
      pltpu.make_async_copy(k_hbm.at[0, 0], kbuf.at[slot], ksem.at[slot]).wait()

      @pl.when(more)
      def _():
        kv_issue(nxt, nslot, 0, NI // 2)

      if mode == 'full':
        s = lax.dot_general(q, kbuf[slot], (((1,), (1,)), ((), ())), preferred_element_type=f32) * scale
        m = jnp.max(s, axis=-1, keepdims=True)
        p = jnp.exp(s - m)
        l = jnp.sum(p, axis=-1, keepdims=True)
        pb = p.astype(bf16)
      pltpu.make_async_copy(v_hbm.at[0, 0], vbuf.at[slot], vsem.at[slot]).wait()

      @pl.when(more)
      def _():
        kv_issue(nxt, nslot, NI // 2, NI)

      if mode == 'full':
        o = jnp.dot(pb, vbuf[slot], preferred_element_type=f32) / l
        row = lax.broadcasted_iota(jnp.int32, o.shape, 0)
        o_scr[h] = jnp.where(row == b, o, o_scr[h])

      for u in range(NU):
        @pl.when(step == U0 + u * US)
        def _():
          late_unit(u)

      @pl.when(step == F0)
      def _():
        pltpu.make_async_copy(wo_hbm, wo_buf, wsem.at[1]).wait()
        pltpu.make_async_copy(wg_hbm, wg_buf, wsem.at[1]).wait()
        pltpu.make_async_copy(wu_hbm, wu_buf, wsem.at[1]).wait()
        pltpu.make_async_copy(wd_hbm, wd_buf, wsem.at[1]).wait()

      @pl.when(b == B - 1)
      def _():
        w = wo_buf[pl.ds(pl.multiple_of(h * Dh, Dh), Dh), :]
        a_acc[...] += jnp.dot(o_scr[h].astype(bf16), w, preferred_element_type=f32)

      @pl.when(jnp.logical_and(step >= F0, step < F0 + NF))
      def _():
        c0 = pl.multiple_of((step - F0) * FC, FC)
        xb = x_ref[...]
        gg = jnp.dot(xb, wg_buf[:, pl.ds(c0, FC)], preferred_element_type=f32)
        uu = jnp.dot(xb, wu_buf[:, pl.ds(c0, FC)], preferred_element_type=f32)
        hid = (gg * _sigmoid(gg)) * uu
        y_acc[...] += jnp.dot(hid.astype(bf16), wd_buf[pl.ds(c0, FC), :], preferred_element_type=f32)
      return carry

    lax.fori_loop(0, NSTEP, body, 0)

    xa = x_ref[...].astype(f32)
    gw = gw_ref[...].astype(f32).reshape(1, D)
    wr = wr_ref[...].astype(f32).reshape(1, D)
    gate = _sigmoid(jnp.sum(xa * gw, axis=-1, keepdims=True))
    r = jnp.sum(xa * wr, axis=-1, keepdims=True)
    y = y_acc[...] * _sigmoid(r)
    bb = xa + (xa * 0.0 + y)
    out_ref[...] = (gate * a_acc[...] + (1.0 - gate) * bb).astype(out_ref.dtype)

  vm = pl.BlockSpec(memory_space=pltpu.VMEM)
  hbm = pl.BlockSpec(memory_space=pl.ANY)
  out = pl.pallas_call(
      kernel,
      in_specs=[vm, vm, vm] + [hbm] * 7,
      out_specs=vm,
      out_shape=jax.ShapeDtypeStruct((B, D), A_x.dtype),
      scratch_shapes=[
          pltpu.VMEM((NS, Sk, Dh), bf16), pltpu.VMEM((NS, Sk, Dh), bf16),
          pltpu.VMEM((D, H * Dh), bf16), pltpu.VMEM((H * Dh, D), bf16),
          pltpu.VMEM((D, F), bf16), pltpu.VMEM((D, F), bf16), pltpu.VMEM((F, D), bf16),
          pltpu.VMEM((H, B, Dh), f32), pltpu.VMEM((H, B, Dh), f32),
          pltpu.VMEM((B, D), f32), pltpu.VMEM((B, D), f32),
          pltpu.SemaphoreType.DMA((NS,)), pltpu.SemaphoreType.DMA((NS,)), pltpu.SemaphoreType.DMA((2,)),
      ],
      compiler_params=pltpu.CompilerParams(vmem_limit_bytes=110 * 1024 * 1024),
  )(A_x.reshape(B, D), B_w_r, gate_w, A_k_cache, A_v_cache, A_wq, A_wo, B_w_gate, B_w_up, B_w_down)
  return out.reshape(B, Sq, D)
```

```python
import jax
import jax.numpy as jnp
from jax import lax
import jax.experimental.pallas as pl
import jax.experimental.pallas.tpu as pltpu

NS = 3
CH = (192, 64)
R = 4
FC = 512
U0, US = 2, 4
NU = 8
F0 = U0 + NU * US + NS


def _sigmoid(z):
    return 1.0 / (1.0 + jnp.exp(-z))


@jax.jit
def pallas_gated_mix__mha_block_cached__moe_arch_mod__decode_kernel(
    A_x, A_k_cache, A_v_cache, A_wq, A_wo, B_x, B_w_r, B_w_gate, B_w_up, B_w_down, gate_w,
):
    del B_x
    B, Sq, D = A_x.shape
    _, H, Sk, Dh = A_k_cache.shape
    F = B_w_gate.shape[1]
    assert (B, Sq, D, H, Sk, Dh, F) == (4, 1, 1024, 32, 8192, 128, 3584)
    NSTEP = B * H
    NF = F // FC
    RR = Sk // R
    PER = sum(CH)
    NI = RR // PER
    scale = Dh ** -0.5
    f32, bf16 = jnp.float32, jnp.bfloat16

    def kernel(x_hbm, wr_hbm, gw_hbm, k_hbm, v_hbm, wq_hbm, wo_hbm, wg_hbm, wu_hbm, wd_hbm,
               out_ref, kbuf, vbuf, wq_buf, wo_buf, wg_buf, wu_buf, wd_buf,
               q_scr, o_scr, a_acc, y_acc, x_ref, wr_ref, gw_ref, ksem, vsem, wsem, ssem):

        def kv_issue(step, slot, lo, hi):
            h = step % H
            b = step // H
            for i in range(lo, hi):
                o0 = 0
                for n in CH:
                    for g in range(R):
                        rows = pl.ds(g * RR + i * PER + o0, n)
                        pltpu.make_async_copy(
                            k_hbm.at[b, h, rows], kbuf.at[slot, rows], ksem.at[slot]).start(priority=0)
                        pltpu.make_async_copy(
                            v_hbm.at[b, h, rows], vbuf.at[slot, rows], vsem.at[slot]).start(priority=1)
                    o0 += n

        def last_issue(src, dst, sem):
            slot = (NSTEP - 1) % NS

            def it(i, c):
                o0 = 0
                for n in CH:
                    for g in range(R):
                        rows = pl.ds(pl.multiple_of(g * RR + i * PER + o0, 16), n)
                        pltpu.make_async_copy(
                            src.at[B - 1, H - 1, rows], dst.at[slot, rows], sem.at[slot]).start(priority=g % 2)
                    o0 += n
                return c
            lax.fori_loop(0, NI, it, 0)

        def weight_unit(pair, starts, region, slab, pieces, sem, nreg=R):
            def it(i, c):
                for dr, nr, c0, nc in pieces:
                    for g in range(nreg):
                        for t in range(2):
                            src, dst = pair[t]
                            rows = pl.ds(pl.multiple_of(starts[t] + g * region + i * slab + dr, 8), nr)
                            cols = pl.ds(c0, nc)
                            pltpu.make_async_copy(src.at[rows, cols], dst.at[rows, cols], sem).start(priority=t)
                return c
            lax.fori_loop(0, region // slab, it, 0)

        row_pieces = ((0, 24, 0, D), (24, 8, 0, D))

        def late_unit(u):
            sem = wsem.at[1]
            if u < 2:
                weight_unit(((wo_hbm, wo_buf),) * 2, (u * 2048, u * 2048 + 1024), 256, 32, row_pieces, sem)
            elif u < 6:
                weight_unit(((wg_hbm, wg_buf), (wu_hbm, wu_buf)), ((u - 2) * 256,) * 2, 64, 8,
                            ((0, 8, 0, 2560), (0, 8, 2560, 1024)), sem)
            elif u == 6:
                weight_unit(((wd_hbm, wd_buf),) * 2, (0, 1024), 256, 32, row_pieces, sem)
            else:
                weight_unit(((wd_hbm, wd_buf),) * 2, (2048, 2816), 256, 32, row_pieces, sem, nreg=3)

        for u in range(2):
            weight_unit(((wq_hbm, wq_buf),) * 2, (u * 512, u * 512 + 256), 64, 8,
                        ((0, 8, 0, 3072), (0, 8, 3072, 1024)), wsem.at[0])
        small = [pltpu.make_async_copy(s, d, ssem.at[i])
                 for i, (s, d) in enumerate(((x_hbm, x_ref), (wr_hbm, wr_ref), (gw_hbm, gw_ref)))]
        for cp in small:
            cp.start()

        def pro(step, c):
            kv_issue(step, step, 0, NI)
            return c
        lax.fori_loop(0, NS - 1, pro, 0)

        a_acc[...] = jnp.zeros_like(a_acc)
        y_acc[...] = jnp.zeros_like(y_acc)
        o_scr[...] = jnp.zeros_like(o_scr)
        for cp in small:
            cp.wait()
        pltpu.make_async_copy(wq_hbm, wq_buf, wsem.at[0]).wait()
        x = x_ref[...]
        for hh in range(H):
            q_scr[hh] = jnp.dot(x, wq_buf[:, hh * Dh:(hh + 1) * Dh], preferred_element_type=f32)

        def body(step, carry):
            h = step % H
            b = step // H
            slot = step % NS
            nxt = step + NS - 1
            nslot = nxt % NS

            q = q_scr[h].astype(bf16)
            pltpu.make_async_copy(k_hbm.at[0, 0], kbuf.at[slot], ksem.at[slot]).wait()

            @pl.when(nxt < NSTEP - 1)
            def _():
                kv_issue(nxt, nslot, 0, NI // 2)

            @pl.when(nxt == NSTEP - 1)
            def _():
                last_issue(k_hbm, kbuf, ksem)

            s = lax.dot_general(q, kbuf[slot], (((1,), (1,)), ((), ())), preferred_element_type=f32) * scale
            m = jnp.max(s, axis=-1, keepdims=True)
            p = jnp.exp(s - m)
            l = jnp.sum(p, axis=-1, keepdims=True)
            pb = p.astype(bf16)
            pltpu.make_async_copy(v_hbm.at[0, 0], vbuf.at[slot], vsem.at[slot]).wait()

            @pl.when(nxt < NSTEP - 1)
            def _():
                kv_issue(nxt, nslot, NI // 2, NI)

            @pl.when(nxt == NSTEP - 1)
            def _():
                last_issue(v_hbm, vbuf, vsem)

            o = jnp.dot(pb, vbuf[slot], preferred_element_type=f32) / l
            row = lax.broadcasted_iota(jnp.int32, o.shape, 0)
            o_scr[h] = jnp.where(row == b, o, o_scr[h])

            for u in range(NU):
                @pl.when(step == U0 + u * US)
                def _():
                    late_unit(u)

            @pl.when(step == F0)
            def _():
                for src, dst in ((wo_hbm, wo_buf), (wg_hbm, wg_buf), (wu_hbm, wu_buf), (wd_hbm, wd_buf)):
                    pltpu.make_async_copy(src, dst, wsem.at[1]).wait()

            @pl.when(b == B - 1)
            def _():
                w = wo_buf[pl.ds(pl.multiple_of(h * Dh, Dh), Dh), :]
                a_acc[...] += jnp.dot(o_scr[h].astype(bf16), w, preferred_element_type=f32)

            @pl.when(jnp.logical_and(step >= F0, step < F0 + NF))
            def _():
                c0 = pl.multiple_of((step - F0) * FC, FC)
                xb = x_ref[...]
                gg = jnp.dot(xb, wg_buf[:, pl.ds(c0, FC)], preferred_element_type=f32)
                uu = jnp.dot(xb, wu_buf[:, pl.ds(c0, FC)], preferred_element_type=f32)
                hid = (gg * _sigmoid(gg)) * uu
                y_acc[...] += jnp.dot(hid.astype(bf16), wd_buf[pl.ds(c0, FC), :], preferred_element_type=f32)
            return carry

        lax.fori_loop(0, NSTEP, body, 0)

        xa = x_ref[...].astype(f32)
        gw = gw_ref[...].astype(f32).reshape(1, D)
        wr = wr_ref[...].astype(f32).reshape(1, D)
        gate = _sigmoid(jnp.sum(xa * gw, axis=-1, keepdims=True))
        r = jnp.sum(xa * wr, axis=-1, keepdims=True)
        y = y_acc[...] * _sigmoid(r)
        bb = xa + (xa * 0.0 + y)
        out_ref[...] = (gate * a_acc[...] + (1.0 - gate) * bb).astype(out_ref.dtype)

    out = pl.pallas_call(
        kernel,
        in_specs=[pl.BlockSpec(memory_space=pl.ANY)] * 10,
        out_specs=pl.BlockSpec(memory_space=pltpu.VMEM),
        out_shape=jax.ShapeDtypeStruct((B, D), A_x.dtype),
        scratch_shapes=[
            pltpu.VMEM((NS, Sk, Dh), bf16), pltpu.VMEM((NS, Sk, Dh), bf16),
            pltpu.VMEM((D, H * Dh), bf16), pltpu.VMEM((H * Dh, D), bf16),
            pltpu.VMEM((D, F), bf16), pltpu.VMEM((D, F), bf16), pltpu.VMEM((F, D), bf16),
            pltpu.VMEM((H, B, Dh), f32), pltpu.VMEM((H, B, Dh), f32),
            pltpu.VMEM((B, D), f32), pltpu.VMEM((B, D), f32),
            pltpu.VMEM((B, D), bf16), pltpu.VMEM((D,), bf16), pltpu.VMEM((D,), bf16),
            pltpu.SemaphoreType.DMA((NS,)), pltpu.SemaphoreType.DMA((NS,)),
            pltpu.SemaphoreType.DMA((2,)), pltpu.SemaphoreType.DMA((3,)),
        ],
        compiler_params=pltpu.CompilerParams(vmem_limit_bytes=96 * 1024 * 1024),
    )(A_x.reshape(B, D), B_w_r, gate_w, A_k_cache, A_v_cache, A_wq, A_wo, B_w_gate, B_w_up, B_w_down)
    return out.reshape(B, Sq, D)
```
